```python
import os as _os
_os.environ.setdefault("JAX_PLATFORMS", "cpu")
import jax
import jax.numpy as jnp

def _softmax(x, axis=-1):
    return jax.nn.softmax(x, axis=axis)
def _gelu(x):
    return jax.nn.gelu(x, approximate=True)
def _silu(x):
    return jax.nn.silu(x)
def _sigmoid(x):
    return jax.nn.sigmoid(x)
def _layernorm(x, axis=-1, eps=1e-5):
    m = jnp.mean(x, axis=axis, keepdims=True)
    v = jnp.var(x, axis=axis, keepdims=True)
    return (x - m) / jnp.sqrt(v + eps)
def _scatter_add(tgt, idx, src, axis=0):
    return tgt.at[idx].add(src)
def _segment_sum(src, seg, n):
    return jax.ops.segment_sum(src, seg, n)
class _Rng:
    def __init__(self, key):
        self._k = key
    def _next(self):
        self._k, sub = jax.random.split(self._k)
        return sub
    def normal(self, shape):
        return jax.random.normal(self._next(), shape, dtype=jnp.bfloat16)
    def randint(self, lo, hi, shape):
        return jax.random.randint(self._next(), shape, lo, hi, dtype=jnp.int32)
    def uniform(self, shape, lo=0.0, hi=1.0):
        return jax.random.uniform(self._next(), shape, jnp.bfloat16, lo, hi)
    def permutation(self, n):
        return jax.random.permutation(self._next(), n)


kernel_name = 'concat_heads__mha_block_cached__mha_block_cached__near_ridge'

def setup_inputs():
    _rng = _Rng(jax.random.key(int.from_bytes(__import__("os").urandom(4), "little")))
    _w = (lambda a: (lambda t: t.astype(jnp.bfloat16) if jnp.issubdtype(t.dtype, jnp.floating) else t)(jnp.asarray(a)))
    def _A_setup():
        B, Sq, D = 8, 144, 640
        H, Sk, Dh = 32, 512, 128
        return {
            "x": _w((lambda *s: _rng.normal(s) * 0.8)(B, Sq, D)),
            "k_cache": _w((lambda *s: _rng.normal(s) * 0.8)(B, H, Sk, Dh)),
            "v_cache": _w((lambda *s: _rng.normal(s) * 0.05)(B, H, Sk, Dh)),
            "wq": _w((lambda *s: _rng.normal(s) * 0.8)(D, H * Dh) * (D ** -0.5)),
            "wo": _w((lambda *s: _rng.normal(s) * 0.05)(H * Dh, D) * ((H * Dh) ** -0.5)),
        }
    _A_in = _A_setup()

    def _B_setup():
        B, Sq, D = 8, 144, 640
        H, Sk, Dh = 32, 512, 128
        return {
            "x": _w((lambda *s: _rng.normal(s) * 0.8)(B, Sq, D)),
            "k_cache": _w((lambda *s: _rng.normal(s) * 0.8)(B, H, Sk, Dh)),
            "v_cache": _w((lambda *s: _rng.normal(s) * 0.05)(B, H, Sk, Dh)),
            "wq": _w((lambda *s: _rng.normal(s) * 0.8)(D, H * Dh) * (D ** -0.5)),
            "wo": _w((lambda *s: _rng.normal(s) * 0.05)(H * Dh, D) * ((H * Dh) ** -0.5)),
        }
    _B_in = _B_setup()

    return {
        "A_x": _A_in["x"],
        "A_k_cache": _A_in["k_cache"],
        "A_v_cache": _A_in["v_cache"],
        "A_wq": _A_in["wq"],
        "A_wo": _A_in["wo"],
        "B_x": _B_in["x"],
        "B_k_cache": _B_in["k_cache"],
        "B_v_cache": _B_in["v_cache"],
        "B_wq": _B_in["wq"],
        "B_wo": _B_in["wo"],
    }

def reference(A_x, A_k_cache, A_v_cache, A_wq, A_wo, B_x, B_k_cache, B_v_cache, B_wq, B_wo):
    def _A_ref(x, k_cache, v_cache, wq, wo):
        B, Sq, D = x.shape
        H, Dh = 32, 128
        q = (lambda x, *d: x.transpose(*d))((x @ wq).reshape(B, Sq, H, Dh), 0, 2, 1, 3)
        scores = jnp.einsum("bhqd,bhkd->bhqk", q, k_cache) * (Dh ** -0.5)
        p = _softmax(scores, axis=-1)
        o = jnp.einsum("bhqk,bhkd->bhqd", p, v_cache)
        return (lambda x, *d: x.transpose(*d))(o, 0, 2, 1, 3).reshape(B, Sq, H * Dh) @ wo

    def _B_ref(x, k_cache, v_cache, wq, wo):
        B, Sq, D = x.shape
        H, Dh = 32, 128
        q = (lambda x, *d: x.transpose(*d))((x @ wq).reshape(B, Sq, H, Dh), 0, 2, 1, 3)
        scores = jnp.einsum("bhqd,bhkd->bhqk", q, k_cache) * (Dh ** -0.5)
        p = _softmax(scores, axis=-1)
        o = jnp.einsum("bhqk,bhkd->bhqd", p, v_cache)
        return (lambda x, *d: x.transpose(*d))(o, 0, 2, 1, 3).reshape(B, Sq, H * Dh) @ wo

    a = _A_ref(A_x, A_k_cache, A_v_cache, A_wq, A_wo)
    b = _B_ref(B_x, B_k_cache, B_v_cache, B_wq, B_wo)
    return jnp.concatenate([a, b], axis=-1)
```

```python
import functools
import jax
import jax.numpy as jnp
import jax.experimental.pallas as pl
import jax.experimental.pallas.tpu as pltpu

B, SQ, D = 8, 144, 640
H, SK, DH = 32, 512, 128
HG = 8
NHG = H // HG
SCALE = DH ** -0.5
NT = (((1,), (1,)), ((), ()))


def _attn_step(b, hg, x_ref, k_ref, v_ref, wq_ref, wo_ref, out_ref, acc_ref, ocol):
    x_b = x_ref[b]
    q = jnp.dot(x_b, wq_ref[...], preferred_element_type=jnp.float32)
    q = (q * SCALE).astype(jnp.bfloat16)
    os_ = []
    for h in range(HG):
        qh = q[:, h * DH:(h + 1) * DH]
        kh = k_ref[0, h]
        s = jax.lax.dot_general(qh, kh, NT, preferred_element_type=jnp.float32)
        m = jnp.max(s, axis=-1, keepdims=True)
        p = jnp.exp(s - m)
        l = jnp.sum(p, axis=-1, keepdims=True)
        o = jnp.dot(p.astype(jnp.bfloat16), v_ref[0, h], preferred_element_type=jnp.float32)
        o = o * (1.0 / l)
        os_.append(o.astype(jnp.bfloat16))
    o_all = jnp.concatenate(os_, axis=1)
    contrib = jnp.dot(o_all, wo_ref[...], preferred_element_type=jnp.float32)

    @pl.when(hg == 0)
    def _():
        acc_ref[b] = contrib

    @pl.when(hg > 0)
    def _():
        acc_ref[b] += contrib

    @pl.when(hg == NHG - 1)
    def _():
        out_ref[b] = acc_ref[b].astype(out_ref.dtype)


def _kernel(ax, ak, av, awq, awo, bx, bk, bv, bwq, bwo, out_ref, acc_ref):
    blk = pl.program_id(0)
    hg = pl.program_id(1)
    b = pl.program_id(2)

    @pl.when(blk == 0)
    def _():
        _attn_step(b, hg, ax, ak, av, awq, awo, out_ref, acc_ref, 0)

    @pl.when(blk == 1)
    def _():
        _attn_step(b, hg, bx, bk, bv, bwq, bwo, out_ref, acc_ref, 1)


@jax.jit
def pallas_concat_heads__mha_block_cached__mha_block_cached__near_ridge_kernel(
    A_x, A_k_cache, A_v_cache, A_wq, A_wo, B_x, B_k_cache, B_v_cache, B_wq, B_wo):

    def specs(which):
        def sel(blk, a_val, b_val):
            return jnp.where(blk == which, a_val, b_val)
        if which == 0:
            kv_map = lambda blk, hg, b: (jnp.where(blk == 0, b, B - 1), jnp.where(blk == 0, hg, NHG - 1), 0, 0)
            wq_map = lambda blk, hg, b: (0, jnp.where(blk == 0, hg, NHG - 1))
            wo_map = lambda blk, hg, b: (jnp.where(blk == 0, hg, NHG - 1), 0)
        else:
            kv_map = lambda blk, hg, b: (jnp.where(blk == 1, b, 0), jnp.where(blk == 1, hg, 0), 0, 0)
            wq_map = lambda blk, hg, b: (0, jnp.where(blk == 1, hg, 0))
            wo_map = lambda blk, hg, b: (jnp.where(blk == 1, hg, 0), 0)
        return [
            pl.BlockSpec((B, SQ, D), lambda blk, hg, b: (0, 0, 0)),
            pl.BlockSpec((1, HG, SK, DH), kv_map),
            pl.BlockSpec((1, HG, SK, DH), kv_map),
            pl.BlockSpec((D, HG * DH), wq_map),
            pl.BlockSpec((HG * DH, D), wo_map),
        ]

    return pl.pallas_call(
        _kernel,
        grid=(2, NHG, B),
        in_specs=specs(0) + specs(1),
        out_specs=pl.BlockSpec((B, SQ, D), lambda blk, hg, b: (0, 0, blk)),
        out_shape=jax.ShapeDtypeStruct((B, SQ, 2 * D), jnp.bfloat16),
        scratch_shapes=[pltpu.VMEM((B, SQ, D), jnp.float32)],
        compiler_params=pltpu.CompilerParams(
            dimension_semantics=("arbitrary", "arbitrary", "arbitrary"),
            vmem_limit_bytes=100 * 1024 * 1024),
    )(A_x, A_k_cache, A_v_cache, A_wq, A_wo, B_x, B_k_cache, B_v_cache, B_wq, B_wo)
```

```python
import math

import jax
import jax.numpy as jnp
import jax.experimental.pallas as pl
import jax.experimental.pallas.tpu as pltpu

B, SQ, D = 8, 144, 640
H, SK, DH = 32, 512, 128
HP = 4
R = 2
NSB = H // HP
NS = 2 * NSB
M = B * SQ
QSCALE = (DH ** -0.5) * math.log2(math.e)
NT = (((1,), (1,)), ((), ()))


def _recip(l):
    r = pl.reciprocal(l, approx=True)
    return r * (2.0 - l * r)


def _kernel(ax, ak, av, awq, awo, bx, bk, bv, bwq, bwo, out_ref,
            x_buf, k_buf, v_buf, wq_buf, wo_buf, o_buf, acc_ref,
            sem_x, sem):
    s = pl.program_id(0)
    blk = s // NSB
    hb = s % NSB

    def copies(which, t):
        h0 = (t % NSB) * HP
        slot = t % R
        k_src = (ak if which == 0 else bk).at[:, pl.ds(h0, HP)]
        v_src = (av if which == 0 else bv).at[:, pl.ds(h0, HP)]
        wq_src = (awq if which == 0 else bwq).at[:, pl.ds(h0 * DH, HP * DH)]
        wo_src = (awo if which == 0 else bwo).at[pl.ds(h0 * DH, HP * DH), :]
        return (pltpu.make_async_copy(wq_src, wq_buf.at[slot], sem.at[slot, 0]),
                pltpu.make_async_copy(k_src, k_buf.at[slot], sem.at[slot, 1]),
                pltpu.make_async_copy(v_src, v_buf.at[slot], sem.at[slot, 2]),
                pltpu.make_async_copy(wo_src, wo_buf.at[slot], sem.at[slot, 3]))

    def x_copy(which):
        return pltpu.make_async_copy(ax if which == 0 else bx, x_buf.at[which], sem_x.at[which])

    @pl.when(s == 0)
    def _():
        x_copy(0).start()
        for cp in copies(0, 0):
            cp.start()

    slot = s % R

    @pl.when((s == 0) | (s == NSB))
    def _():
        pltpu.make_async_copy(ax, x_buf.at[blk], sem_x.at[blk]).wait()

    pltpu.make_async_copy(awq.at[:, pl.ds(0, HP * DH)], wq_buf.at[slot], sem.at[slot, 0]).wait()

    q = jnp.dot(x_buf[blk], wq_buf[slot], preferred_element_type=jnp.float32)
    q = (q * QSCALE).astype(jnp.bfloat16)

    pltpu.make_async_copy(ak.at[:, pl.ds(0, HP)], k_buf.at[slot], sem.at[slot, 1]).wait()
    pltpu.make_async_copy(ak.at[:, pl.ds(0, HP)], v_buf.at[slot], sem.at[slot, 2]).wait()

    def issue(t):
        @pl.when(t < NSB)
        def _():
            for cp in copies(0, t):
                cp.start()

        @pl.when((t >= NSB) & (t < NS))
        def _():
            for cp in copies(1, t):
                cp.start()

    issue(s + R - 1)

    @pl.when(s == 1)
    def _():
        x_copy(1).start()

    pairs = [(bi, j) for bi in range(B) for j in range(HP)]

    def qk(i):
        bi, j = pairs[i]
        qh = q[bi * SQ:(bi + 1) * SQ, j * DH:(j + 1) * DH]
        return jax.lax.dot_general(qh, k_buf[slot, bi, j], NT, preferred_element_type=jnp.float32)

    s_next = qk(0)
    for i, (bi, j) in enumerate(pairs):
        s_cur = s_next
        if i + 1 < len(pairs):
            s_next = qk(i + 1)
        m = jnp.max(s_cur, axis=-1, keepdims=True)
        p = jnp.exp2(s_cur - m)
        l = jnp.sum(p, axis=-1, keepdims=True)
        o = jnp.dot(p.astype(jnp.bfloat16), v_buf[slot, bi, j], preferred_element_type=jnp.float32)
        o_buf[bi * SQ:(bi + 1) * SQ, j * DH:(j + 1) * DH] = (o * _recip(l)).astype(jnp.bfloat16)

    pltpu.make_async_copy(awo.at[pl.ds(0, HP * DH), :], wo_buf.at[slot], sem.at[slot, 3]).wait()
    contrib = jnp.dot(o_buf[...], wo_buf[slot], preferred_element_type=jnp.float32)
    acc = jnp.where(hb > 0, acc_ref[...], 0.0) + contrib
    acc_ref[...] = acc
    out_ref[...] = acc.astype(out_ref.dtype)


@jax.jit
def pallas_concat_heads__mha_block_cached__mha_block_cached__near_ridge_kernel(
    A_x: jax.Array,
    A_k_cache: jax.Array,
    A_v_cache: jax.Array,
    A_wq: jax.Array,
    A_wo: jax.Array,
    B_x: jax.Array,
    B_k_cache: jax.Array,
    B_v_cache: jax.Array,
    B_wq: jax.Array,
    B_wo: jax.Array,
):
    any_spec = pl.BlockSpec(memory_space=pl.ANY)
    out = pl.pallas_call(
        _kernel,
        grid=(NS,),
        in_specs=[any_spec] * 10,
        out_specs=pl.BlockSpec((M, D), lambda s: (0, s // NSB)),
        out_shape=jax.ShapeDtypeStruct((M, 2 * D), jnp.bfloat16),
        scratch_shapes=[
            pltpu.VMEM((2, M, D), jnp.bfloat16),
            pltpu.VMEM((R, B, HP, SK, DH), jnp.bfloat16),
            pltpu.VMEM((R, B, HP, SK, DH), jnp.bfloat16),
            pltpu.VMEM((R, D, HP * DH), jnp.bfloat16),
            pltpu.VMEM((R, HP * DH, D), jnp.bfloat16),
            pltpu.VMEM((M, HP * DH), jnp.bfloat16),
            pltpu.VMEM((M, D), jnp.float32),
            pltpu.SemaphoreType.DMA((2,)),
            pltpu.SemaphoreType.DMA((R, 4)),
        ],
        compiler_params=pltpu.CompilerParams(
            dimension_semantics=("arbitrary",),
            vmem_limit_bytes=100 * 1024 * 1024),
    )(A_x.reshape(M, D), A_k_cache, A_v_cache, A_wq, A_wo,
      B_x.reshape(M, D), B_k_cache, B_v_cache, B_wq, B_wo)
    return out.reshape(B, SQ, 2 * D)
```

```python
import math

import jax
import jax.numpy as jnp
import jax.experimental.pallas as pl
import jax.experimental.pallas.tpu as pltpu

B, SQ, D = 8, 144, 640
H, SK, DH = 32, 512, 128
HP = 4
R = 2
NSB = H // HP
NS = 2 * NSB
M = B * SQ
QSCALE = (DH ** -0.5) * math.log2(math.e)
NT = (((1,), (1,)), ((), ()))


def _recip(l):
    r = pl.reciprocal(l, approx=True)
    return r * (2.0 - l * r)


def _kernel(ax, ak, av, awq, awo, bx, bk, bv, bwq, bwo, out_ref,
            x_buf, k_buf, v_buf, wq_buf, wo_buf, q_scr, o_buf, acc_ref,
            sem_x, sem_wq, sem):
    g = pl.program_id(0)

    def wq_copy(which, t):
        src = (awq if which == 0 else bwq).at[:, pl.ds((t % NSB) * HP * DH, HP * DH)]
        return pltpu.make_async_copy(src, wq_buf.at[t % 2], sem_wq.at[t % 2])

    def kvo_copies(which, t):
        h0 = (t % NSB) * HP
        slot = t % R
        return (pltpu.make_async_copy((ak if which == 0 else bk).at[:, pl.ds(h0, HP)],
                                      k_buf.at[slot], sem.at[slot, 0]),
                pltpu.make_async_copy((av if which == 0 else bv).at[:, pl.ds(h0, HP)],
                                      v_buf.at[slot], sem.at[slot, 1]),
                pltpu.make_async_copy((awo if which == 0 else bwo).at[pl.ds(h0 * DH, HP * DH), :],
                                      wo_buf.at[slot], sem.at[slot, 2]))

    def x_copy(which):
        return pltpu.make_async_copy(ax if which == 0 else bx, x_buf.at[which], sem_x.at[which])

    def start_wq(t):
        @pl.when(t < NSB)
        def _():
            wq_copy(0, t).start()

        @pl.when((t >= NSB) & (t < NS))
        def _():
            wq_copy(1, t).start()

    def start_kvo(t):
        @pl.when(t < NSB)
        def _():
            for cp in kvo_copies(0, t):
                cp.start()

        @pl.when((t >= NSB) & (t < NS))
        def _():
            for cp in kvo_copies(1, t):
                cp.start()

    @pl.when(g == 0)
    def _():
        x_copy(0).start()
        wq_copy(0, 0).start()

    @pl.when(g >= 1)
    def _():
        start_wq(g + 1)

    @pl.when(g < NS)
    def _():
        blk_q = g // NSB

        @pl.when((g == 0) | (g == NSB))
        def _():
            pltpu.make_async_copy(ax, x_buf.at[blk_q], sem_x.at[blk_q]).wait()

        pltpu.make_async_copy(awq.at[:, pl.ds(0, HP * DH)], wq_buf.at[g % 2], sem_wq.at[g % 2]).wait()

        @pl.when(g == 0)
        def _():
            for cp in kvo_copies(0, 0):
                cp.start()
            wq_copy(0, 1).start()

        q = jnp.dot(x_buf[blk_q], wq_buf[g % 2], preferred_element_type=jnp.float32)
        q_scr[g % 2] = (q * QSCALE).astype(jnp.bfloat16)

    @pl.when(g >= 1)
    def _():
        a = g - 1
        slot = a % R
        hb = a % NSB
        pltpu.make_async_copy(ak.at[:, pl.ds(0, HP)], k_buf.at[slot], sem.at[slot, 0]).wait()
        pltpu.make_async_copy(ak.at[:, pl.ds(0, HP)], v_buf.at[slot], sem.at[slot, 1]).wait()

        start_kvo(g)

        @pl.when(g == 1)
        def _():
            x_copy(1).start()

        q = q_scr[a % 2]
        pairs = [(bi, j) for bi in range(B) for j in range(HP)]

        def qk(i):
            bi, j = pairs[i]
            return jax.lax.dot_general(q[bi * SQ:(bi + 1) * SQ, j * DH:(j + 1) * DH],
                                       k_buf[slot, bi, j], NT, preferred_element_type=jnp.float32)

        s_next = qk(0)
        for i, (bi, j) in enumerate(pairs):
            s_cur = s_next
            if i + 1 < len(pairs):
                s_next = qk(i + 1)
            m = jnp.max(s_cur, axis=-1, keepdims=True)
            p = jnp.exp2(s_cur - m)
            l = jnp.sum(p, axis=-1, keepdims=True)
            o = jnp.dot(p.astype(jnp.bfloat16), v_buf[slot, bi, j], preferred_element_type=jnp.float32)
            o_buf[bi * SQ:(bi + 1) * SQ, j * DH:(j + 1) * DH] = (o * _recip(l)).astype(jnp.bfloat16)

        pltpu.make_async_copy(awo.at[pl.ds(0, HP * DH), :], wo_buf.at[slot], sem.at[slot, 2]).wait()
        contrib = jnp.dot(o_buf[...], wo_buf[slot], preferred_element_type=jnp.float32)
        acc = jnp.where(hb > 0, acc_ref[...], 0.0) + contrib
        acc_ref[...] = acc
        out_ref[...] = acc.astype(out_ref.dtype)


@jax.jit
def pallas_concat_heads__mha_block_cached__mha_block_cached__near_ridge_kernel(
    A_x: jax.Array,
    A_k_cache: jax.Array,
    A_v_cache: jax.Array,
    A_wq: jax.Array,
    A_wo: jax.Array,
    B_x: jax.Array,
    B_k_cache: jax.Array,
    B_v_cache: jax.Array,
    B_wq: jax.Array,
    B_wo: jax.Array,
):
    any_spec = pl.BlockSpec(memory_space=pl.ANY)
    out = pl.pallas_call(
        _kernel,
        grid=(NS + 1,),
        in_specs=[any_spec] * 10,
        out_specs=pl.BlockSpec((M, D), lambda g: (0, jnp.maximum(g - 1, 0) // NSB)),
        out_shape=jax.ShapeDtypeStruct((M, 2 * D), jnp.bfloat16),
        scratch_shapes=[
            pltpu.VMEM((2, M, D), jnp.bfloat16),
            pltpu.VMEM((R, B, HP, SK, DH), jnp.bfloat16),
            pltpu.VMEM((R, B, HP, SK, DH), jnp.bfloat16),
            pltpu.VMEM((2, D, HP * DH), jnp.bfloat16),
            pltpu.VMEM((R, HP * DH, D), jnp.bfloat16),
            pltpu.VMEM((2, M, HP * DH), jnp.bfloat16),
            pltpu.VMEM((M, HP * DH), jnp.bfloat16),
            pltpu.VMEM((M, D), jnp.float32),
            pltpu.SemaphoreType.DMA((2,)),
            pltpu.SemaphoreType.DMA((2,)),
            pltpu.SemaphoreType.DMA((R, 3)),
        ],
        compiler_params=pltpu.CompilerParams(
            dimension_semantics=("arbitrary",),
            vmem_limit_bytes=100 * 1024 * 1024),
    )(A_x.reshape(M, D), A_k_cache, A_v_cache, A_wq, A_wo,
      B_x.reshape(M, D), B_k_cache, B_v_cache, B_wq, B_wo)
    return out.reshape(B, SQ, 2 * D)
```
